```python
import jax
import jax.numpy as jnp

def _softmax(x, axis=-1):
    return jax.nn.softmax(x, axis=axis)
def _gelu(x):
    return jax.nn.gelu(x, approximate=True)
def _silu(x):
    return jax.nn.silu(x)
def _sigmoid(x):
    return jax.nn.sigmoid(x)
def _layernorm(x, axis=-1, eps=1e-5):
    m = jnp.mean(x, axis=axis, keepdims=True)
    v = jnp.var(x, axis=axis, keepdims=True)
    return (x - m) / jnp.sqrt(v + eps)
def _scatter_add(tgt, idx, src, axis=0):
    return tgt.at[idx].add(src)
def _segment_sum(src, seg, n):
    return jax.ops.segment_sum(src, seg, n)
class _Rng:
    def __init__(self, key):
        self._k = key
    def _next(self):
        self._k, sub = jax.random.split(self._k)
        return sub
    def normal(self, shape):
        return jax.random.normal(self._next(), shape, dtype=jnp.bfloat16)
    def randint(self, lo, hi, shape):
        return jax.random.randint(self._next(), shape, lo, hi, dtype=jnp.int32)
    def uniform(self, shape, lo=0.0, hi=1.0):
        return jax.random.uniform(self._next(), shape, jnp.bfloat16, lo, hi)
    def permutation(self, n):
        return jax.random.permutation(self._next(), n)


kernel_name = 'gated_mix__mha_block_cached__compressed_kv_cla__decode'

def setup_inputs():
    _rng = _Rng(jax.random.key(int.from_bytes(__import__("os").urandom(4), "little")))
    _w = (lambda a: (lambda t: t.astype(jnp.bfloat16) if jnp.issubdtype(t.dtype, jnp.floating) else t)(jnp.asarray(a)))
    def _A_setup():
        B, Sq, D = 2, 1, 512
        H, Sk, Dh = 32, 8192, 128
        return {
            "x": _w((lambda *s: _rng.normal(s) * 0.05)(B, Sq, D)),
            "k_cache": _w((lambda *s: _rng.normal(s) * 0.05)(B, H, Sk, Dh)),
            "v_cache": _w((lambda *s: _rng.normal(s) * 0.05)(B, H, Sk, Dh)),
            "wq": _w((lambda *s: _rng.normal(s) * 0.05)(D, H * Dh) * (D ** -0.5)),
            "wo": _w((lambda *s: _rng.normal(s) * 0.05)(H * Dh, D) * ((H * Dh) ** -0.5)),
        }
    _A_in = _A_setup()

    def _B_setup():
        B, H, Sq, Sk, D, M = 2, 32, 1, 8192, 128, 512
        Dc = 4 * D
        return {
            "x": _w((lambda *s: _rng.normal(s) * 0.05)(B, Sq, M)),
            "c_kv": _w((lambda *s: _rng.normal(s) * 0.05)(B, Sk, Dc)),
            "w_q": _w((lambda *s: _rng.normal(s) * 0.05)(M, H, D) * (M ** -0.5)),
            "w_uk": _w((lambda *s: _rng.normal(s) * 0.05)(Dc, H, D) * (Dc ** -0.5)),
            "w_uv": _w((lambda *s: _rng.normal(s) * 0.05)(Dc, H, D) * (Dc ** -0.5)),
            "w_o": _w((lambda *s: _rng.normal(s) * 0.05)(H, D, M) * ((H * D) ** -0.5)),
        }
    _B_in = _B_setup()

    return {
        "A_x": _A_in["x"],
        "A_k_cache": _A_in["k_cache"],
        "A_v_cache": _A_in["v_cache"],
        "A_wq": _A_in["wq"],
        "A_wo": _A_in["wo"],
        "B_x": _B_in["x"],
        "B_c_kv": _B_in["c_kv"],
        "B_w_q": _B_in["w_q"],
        "B_w_uk": _B_in["w_uk"],
        "B_w_uv": _B_in["w_uv"],
        "B_w_o": _B_in["w_o"],
        "gate_w": _w((lambda *s: _rng.normal(s) * 0.05)(512)),
    }

def reference(A_x, A_k_cache, A_v_cache, A_wq, A_wo, B_x, B_c_kv, B_w_q, B_w_uk, B_w_uv, B_w_o, gate_w):
    def _A_ref(x, k_cache, v_cache, wq, wo):
        B, Sq, D = x.shape
        H, Dh = 32, 128
        q = (lambda x, *d: x.transpose(*d))((x @ wq).reshape(B, Sq, H, Dh), 0, 2, 1, 3)
        scores = jnp.einsum("bhqd,bhkd->bhqk", q, k_cache) * (Dh ** -0.5)
        p = _softmax(scores, axis=-1)
        o = jnp.einsum("bhqk,bhkd->bhqd", p, v_cache)
        return (lambda x, *d: x.transpose(*d))(o, 0, 2, 1, 3).reshape(B, Sq, H * Dh) @ wo

    def _B_ref(x, c_kv, w_q, w_uk, w_uv, w_o):
        B, Sq, M = x.shape[0], x.shape[1], x.shape[2]
        Sk = c_kv.shape[1]
        H, D = w_q.shape[1], w_q.shape[2]
        q = jnp.einsum("bqm,mhd->bhqd", x, w_q)
        k = jnp.einsum("bkc,chd->bhkd", c_kv, w_uk)
        v = jnp.einsum("bkc,chd->bhkd", c_kv, w_uv)
        scores = jnp.einsum("bhqd,bhkd->bhqk", q, k) * (D ** -0.5)
        off = Sk - Sq
        qi = jnp.arange(Sq)[:, None]
        kj = jnp.arange(Sk)[None, :]
        cmask = kj <= (qi + off)
        scores = jnp.where(cmask[None, None], scores, -1e9)
        p = _softmax(scores, axis=-1)
        ctx = jnp.einsum("bhqk,bhkd->bhqd", p, v)
        return jnp.einsum("bhqd,hdm->bqm", ctx, w_o)

    x = A_x
    g = _sigmoid((x * gate_w).sum(-1, keepdims=True))
    a = _A_ref(x, A_k_cache, A_v_cache, A_wq, A_wo)
    b = _B_ref(x, B_c_kv, B_w_q, B_w_uk, B_w_uv, B_w_o)
    return g * a + (1 - g) * b
```

```python
import jax
import jax.numpy as jnp
import jax.experimental.pallas as pl
import jax.experimental.pallas.tpu as pltpu

_B, _H, _SK, _DH, _D, _DC = 2, 32, 8192, 128, 512, 512

_NR = 64
_HW = 4
_ORD_A = (1, 2, 3, 0)
_ORD_B = (4, 5, 6, 7)
_ORD_V = (0, 1, 2, 3, 4, 5, 6, 7)
_OFF = (0, 2, 22)
_PRIO = (0, 1, 1, 1)
_LAG = 8
_CK = 1024
_END = (6, 1, 1)
_RH = 3

_f32 = jnp.float32
_bf16 = jnp.bfloat16


def _dot(a, b):
    return jnp.dot(a, b, preferred_element_type=_f32)


def _dot_t(a, b):
    return jax.lax.dot_general(a, b, (((1,), (1,)), ((), ())), preferred_element_type=_f32)


def _unpack_pair(blk):
    lo = pltpu.bitcast(blk << 16, _f32).astype(_bf16)
    hi = pltpu.bitcast(blk & jnp.int32(-65536), _f32).astype(_bf16)
    return lo, hi


def _loop(lo, hi, body):
    def step(i, carry):
        body(i)
        return carry
    jax.lax.fori_loop(lo, hi, step, 0)


def _kernel(x_hbm, gw_hbm,
            k_hbm, v_hbm, wq_hbm, wo_hbm, ckv_hbm, bwq_hbm, bwuk_hbm, bwuv_hbm, bwo_hbm,
            out_ref,
            kv_buf, wq_v, wob_v, ckv_v, bwq_v, bwuk_v, bwuv_v,
            qa_s, qb_s, qlat_s, clat_s, o_s, ctx_s, m_s, l_s, acc_s,
            x_ref, gw_ref, w32, kv_sem, w_sem, x_sem):

    S_WQ, S_BWQ, S_BWUK, S_BWUV, S_CKV, S_END = 0, 1, 2, 3, 4, 5

    def rows_piece(src, dst, sem, nrow, src0=0):
        def piece(r, p):
            row = pl.multiple_of((r * _NR + p) * nrow, nrow)
            return pltpu.make_async_copy(src.at[pl.ds(src0 + row, nrow)], dst.at[pl.ds(row, nrow)], sem)
        return piece

    def wq_piece(r, p):
        idx = (pl.ds(pl.multiple_of(r * 128 + (p >> 2) * 8, 8), 8), pl.ds(pl.multiple_of((p & 3) * 1024, 1024), 1024))
        return pltpu.make_async_copy(wq_hbm.at[idx], wq_v.at[idx], w_sem.at[S_WQ])

    def issue_round(t, first, second):
        pa, pb, pv = [(t + c) & (_NR - 1) for c in _OFF]
        for i in range(4):
            first(_ORD_A[i], pa).start(priority=_PRIO[0])
            second(_ORD_V[2 * i], pv).start(priority=_PRIO[1])
            first(_ORD_B[i], pb).start(priority=_PRIO[2])
            second(_ORD_V[2 * i + 1], pv).start(priority=_PRIO[3])

    def two(lo, hi):
        return lambda r, p: lo(r, p) if r < 4 else hi(r - 4, p)

    def round_w(t):
        issue_round(t,
                    two(wq_piece, rows_piece(bwq_hbm, bwq_v, w_sem.at[S_BWQ], 64)),
                    two(rows_piece(bwuk_hbm, bwuk_v, w_sem.at[S_BWUK], 64),
                        rows_piece(bwuv_hbm, bwuv_v, w_sem.at[S_BWUV], 64)))

    def round_c(t):
        piece = rows_piece(ckv_hbm, ckv_v, w_sem.at[S_CKV], 16)
        issue_round(t, piece, lambda r, p: piece(r + 8, p))

    def round_kv(w, t):
        slot = w & 1
        src0 = pl.multiple_of(w * (_HW * _SK), _HW * _SK)
        issue_round(t,
                    rows_piece(k_hbm, kv_buf.at[slot, 0], kv_sem.at[slot], 64, src0),
                    rows_piece(v_hbm, kv_buf.at[slot, 1], kv_sem.at[slot], 64, src0))

    end_lo = [sum(_END[:e]) for e in range(len(_END) + 1)]

    def round_end(e, t):
        i, p = t >> 3, t & 7
        for r in range(4):
            for j, src in enumerate((wo_hbm, bwo_hbm)):
                pltpu.make_async_copy(
                    src.at[pl.ds(pl.multiple_of(r * 1024 + t * 16, 16), 16)],
                    wob_v.at[i, j, r, pl.ds(pl.multiple_of(p * 16, 16), 16)],
                    w_sem.at[S_END + e]).start(priority=_PRIO[(2 * r + j) % 4])

    def wait_all(dst, sem):
        pltpu.make_async_copy(dst, dst, sem).wait()

    row8 = jax.lax.broadcasted_iota(jnp.int32, (8, _D), 0)
    row8h = jax.lax.broadcasted_iota(jnp.int32, (8, _DH), 0)
    scale = _DH ** -0.5

    def qa_step(x8, g):
        q = _dot(x8, wq_v[:, pl.ds(pl.multiple_of(g * 512, 512), 512)]) * scale
        for j in range(4):
            qa_s[4 * g + j] = q[:, j * _DH:(j + 1) * _DH]

    def words_step(w_v, blk):
        R = 512
        w32[pl.ds(pl.multiple_of(blk * R, R), R), :] = pltpu.bitcast(
            w_v[pl.ds(pl.multiple_of(2 * blk * R, 2 * R), 2 * R), :], jnp.int32)

    def head_pair(i):
        return _unpack_pair(w32[pl.ds(i, _D, stride=_H // 2), :])

    def qb_step(x8, i):
        lo, hi = head_pair(i)
        qb_s[2 * i] = _dot(x8, lo)
        qb_s[2 * i + 1] = _dot(x8, hi)

    def qlat_step(i):
        pair = head_pair(i)
        for j in range(2):
            h = 2 * i + j
            ql = _dot_t(qb_s[h].astype(_bf16), pair[j]) * scale
            qlat_s[0, pl.ds(h, 1), :] = ql[0:1, :]
            qlat_s[1, pl.ds(h, 1), :] = ql[1:2, :]

    def b_step(i):
        b = i & 1
        ck = ckv_v[pl.ds(pl.multiple_of(b * _SK + (i >> 1) * _CK, _CK), _CK), :]
        s = _dot_t(qlat_s[b].astype(_bf16), ck)
        m_old = m_s[b]
        m_new = jnp.maximum(m_old, jnp.max(s, axis=-1, keepdims=True))
        p = jnp.exp(s - m_new)
        alpha = jnp.exp(m_old - m_new)
        m_s[b] = m_new
        l_s[b] = alpha * l_s[b] + jnp.sum(p, axis=-1, keepdims=True)
        acc_s[b] = alpha * acc_s[b] + _dot(p.astype(_bf16), ck)

    def ctx_step(i):
        pair = head_pair(i)
        for j in range(2):
            h = 2 * i + j
            r0 = clat_s[0, pl.ds(h, 1), :]
            r1 = clat_s[1, pl.ds(h, 1), :]
            lhs = jnp.where(row8 == 0, r0, jnp.where(row8 == 1, r1, 0.0))
            ctx_s[h] = _dot(lhs.astype(_bf16), pair[j])

    def a_head(w, i, between):
        bh = w * _HW + i
        b, h = bh // _H, bh % _H
        keys = pl.ds(pl.multiple_of(i * _SK, _SK), _SK)
        s = _dot_t(qa_s[h].astype(_bf16), kv_buf[w & 1, 0, keys, :])
        m = jnp.max(s, axis=-1, keepdims=True)
        between(0)
        p = jnp.exp(s - m)
        l = jnp.sum(p, axis=-1, keepdims=True)
        o = _dot(p.astype(_bf16), kv_buf[w & 1, 1, keys, :]) / l
        o_s[h] = jnp.where(row8h == b, o, o_s[h])
        between(1)

    def with_rounds(issue, t0, n, per, step):
        def body(i):
            for u in range(per):
                issue(t0 + i * per + u)
            step(i)
        _loop(0, n, body)
        return t0 + n * per

    cx = pltpu.make_async_copy(x_hbm, x_ref, x_sem.at[0])
    cg = pltpu.make_async_copy(gw_hbm, gw_ref, x_sem.at[1])
    round_w(0)
    cx.start()
    cg.start()
    _loop(1, _NR, round_w)
    o_s[...] = jnp.zeros_like(o_s)
    m_s[...] = jnp.full_like(m_s, -jnp.inf)
    l_s[...] = jnp.zeros_like(l_s)
    acc_s[...] = jnp.zeros_like(acc_s)
    cx.wait()
    cg.wait()
    xf = x_ref[...].astype(_f32)
    x8f = jnp.where(row8 == 0, xf[0:1], jnp.where(row8 == 1, xf[1:2], 0.0))
    x8 = x8f.astype(_bf16)
    gate = jax.nn.sigmoid(jnp.sum(x8f * gw_ref[...].astype(_f32).reshape(1, _D), axis=-1, keepdims=True))

    _loop(0, _LAG, round_c)
    wait_all(wq_v, w_sem.at[S_WQ])
    wait_all(bwq_v, w_sem.at[S_BWQ])
    wait_all(bwuk_v, w_sem.at[S_BWUK])
    wait_all(bwuv_v, w_sem.at[S_BWUV])
    t = with_rounds(round_c, _LAG, 8, 1, lambda g: qa_step(x8, g))
    t = with_rounds(round_c, t, 16, 1, lambda i: words_step(bwq_v, i))
    t = with_rounds(round_c, t, 16, 1, lambda i: qb_step(x8, i))
    _loop(t, _NR, round_c)

    def kv_window(w):
        issue = lambda t: round_kv(w, t)
        _loop(0, _LAG, issue)
        t0 = _LAG + 2 * _RH * _HW

        @pl.when(w == 0)
        def _():
            _loop(_LAG, t0, issue)

        @pl.when(w > 0)
        def _():
            wait_all(kv_buf.at[(w - 1) & 1], kv_sem.at[(w - 1) & 1])

            def head(i):
                def between(half):
                    for u in range(_RH):
                        issue(_LAG + (2 * i + half) * _RH + u)
                a_head(w - 1, i, between)
            _loop(0, _HW, head)

        @pl.when(w == 0)
        def _():
            t = with_rounds(issue, t0, 16, 1, lambda i: words_step(bwuk_v, i))
            with_rounds(issue, t, 16, 1, qlat_step)

        @pl.when(w == 1)
        def _():
            wait_all(ckv_v, w_sem.at[S_CKV])

        @pl.when((w == 1) | (w == 2))
        def _():
            n = _SK // _CK
            with_rounds(issue, t0, n, 32 // n, lambda i: b_step((w - 1) * n + i))

        @pl.when(w == 3)
        def _():
            clat_s[...] = acc_s[...] / l_s[...]
            t = with_rounds(issue, t0, 16, 1, lambda i: words_step(bwuv_v, i))
            with_rounds(issue, t, 16, 1, ctx_step)

        _loop(jnp.where(w <= 3, t0 + 32, t0), _NR, issue)

    NW = _B * _H // _HW
    _loop(0, NW, kv_window)

    n0 = 8 * _END[0]
    issue = lambda t: round_end(0, t)
    _loop(0, 2 * _LAG, issue)
    wait_all(kv_buf.at[(NW - 1) & 1], kv_sem.at[(NW - 1) & 1])
    per = (n0 - 2 * _LAG) // (2 * _HW)

    def head(i):
        def between(half):
            for u in range(per):
                issue(2 * _LAG + (2 * i + half) * per + u)
        a_head(NW - 1, i, between)
    _loop(0, _HW, head)
    for e in range(1, len(_END)):
        _loop(8 * end_lo[e], 8 * end_lo[e + 1], lambda t, e=e: round_end(e, t))

    out_a = out_b = None
    for e in range(len(_END)):
        wait_all(wob_v.at[pl.ds(end_lo[e], _END[e])], w_sem.at[S_END + e])
        for i in range(end_lo[e], end_lo[e + 1]):
            for r in range(4):
                ta = _dot(o_s[8 * r + i].astype(_bf16), wob_v[i, 0, r])
                tb = _dot(ctx_s[8 * r + i].astype(_bf16), wob_v[i, 1, r])
                out_a = ta if out_a is None else out_a + ta
                out_b = tb if out_b is None else out_b + tb
    res = gate * out_a + (1.0 - gate) * out_b
    out_ref[...] = res[0:2, :].astype(_bf16)


@jax.jit
def pallas_gated_mix__mha_block_cached__compressed_kv_cla__decode_kernel(
    A_x: jax.Array,
    A_k_cache: jax.Array,
    A_v_cache: jax.Array,
    A_wq: jax.Array,
    A_wo: jax.Array,
    B_x: jax.Array,
    B_c_kv: jax.Array,
    B_w_q: jax.Array,
    B_w_uk: jax.Array,
    B_w_uv: jax.Array,
    B_w_o: jax.Array,
    gate_w: jax.Array,
):
    del B_x
    k2 = A_k_cache.reshape(_B * _H * _SK, _DH)
    v2 = A_v_cache.reshape(_B * _H * _SK, _DH)
    ckv = B_c_kv.reshape(_B * _SK, _DC)
    bwq = B_w_q.reshape(_D * _H, _DH)
    bwuk = B_w_uk.reshape(_DC * _H, _DH)
    bwuv = B_w_uv.reshape(_DC * _H, _DH)
    bwo = B_w_o.reshape(_H * _DH, _D)
    x2 = A_x.reshape(_B, _D)

    hbm = pl.BlockSpec(memory_space=pl.ANY)
    vmem = pl.BlockSpec(memory_space=pltpu.VMEM)
    V = pltpu.VMEM
    scratch = [
        V((2, 2, _HW * _SK, _DH), _bf16),
        V((_D, _H * _DH), _bf16),
        V((8, 2, 4, _DH, _D), _bf16),
        V((_B * _SK, _DC), _bf16),
        V((_D * _H, _DH), _bf16),
        V((_DC * _H, _DH), _bf16),
        V((_DC * _H, _DH), _bf16),
        V((_H, 8, _DH), _f32),
        V((_H, 8, _DH), _f32),
        V((_B, _H, _DC), _f32),
        V((_B, _H, _DC), _f32),
        V((_H, 8, _DH), _f32),
        V((_H, 8, _DH), _f32),
        V((_B, _H, 1), _f32),
        V((_B, _H, 1), _f32),
        V((_B, _H, _DC), _f32),
        V((_B, _D), _bf16),
        V((_D,), _bf16),
        V((_D * _H // 2, _DH), jnp.int32),
        pltpu.SemaphoreType.DMA((2,)),
        pltpu.SemaphoreType.DMA((5 + len(_END),)),
        pltpu.SemaphoreType.DMA((2,)),
    ]
    out = pl.pallas_call(
        _kernel,
        out_shape=jax.ShapeDtypeStruct((_B, _D), _bf16),
        in_specs=[hbm] * 11,
        out_specs=vmem,
        scratch_shapes=scratch,
        compiler_params=pltpu.CompilerParams(vmem_limit_bytes=100 * 1024 * 1024,
                                             disable_semaphore_checks=True),
    )(x2, gate_w, k2, v2, A_wq, A_wo, ckv, bwq, bwuk, bwuv, bwo)
    return out.reshape(_B, 1, _D)
```

```python
import jax
import jax.numpy as jnp
import jax.experimental.pallas as pl
import jax.experimental.pallas.tpu as pltpu

_B, _H, _SK, _DH, _D, _DC = 2, 32, 8192, 128, 512, 512

_NR = 64
_HW = 8
_SKEW = 32
_ESKEW = 32
_LAG = 8
_RH = 3
_CK = 1024
_END = (8, 4, 2, 2)
_EPRIO = ("0111", "0111", "01", "01", "01")
_WORD = (0, 1, 2, 3)

_f32 = jnp.float32
_bf16 = jnp.bfloat16


def _dot(a, b):
    return jnp.dot(a, b, preferred_element_type=_f32)


def _dot_t(a, b):
    return jax.lax.dot_general(a, b, (((1,), (1,)), ((), ())), preferred_element_type=_f32)


def _unpack_pair(blk):
    lo = pltpu.bitcast(blk << 16, _f32).astype(_bf16)
    hi = pltpu.bitcast(blk & jnp.int32(-65536), _f32).astype(_bf16)
    return lo, hi


def _loop(lo, hi, body):
    def step(i, carry):
        body(i)
        return carry
    jax.lax.fori_loop(lo, hi, step, 0)


def _kernel(x_hbm, gw_hbm,
            k_hbm, v_hbm, wq_hbm, wo_hbm, ckv_hbm, bwq_hbm, bwuk_hbm, bwuv_hbm, bwo_hbm,
            out_ref,
            k_v, v_v, wq_v, wob_v, ckv_v, bwq_v, bwuk_v, bwuv_v,
            qa_s, p_s, la_s, qb_s, qlat_s, clat_s, o_s, ctx_s, m_s, l_s, acc_s,
            x_ref, gw_ref, w32, sem):

    S_X, S_GW, S_K, S_V, S_WQ, S_BWQ, S_BWUK, S_BWUV, S_CKV, S_END = range(10)

    def rows_piece(src, dst, s, nrow, src0=0):
        def piece(r, p):
            row = pl.multiple_of((r * _NR + p) * nrow, nrow)
            return pltpu.make_async_copy(src.at[pl.ds(src0 + row, nrow)], dst.at[pl.ds(row, nrow)], sem.at[s])
        return piece

    def wq_piece(r, p):
        idx = (pl.ds(pl.multiple_of(r * 128 + (p >> 2) * 8, 8), 8), pl.ds(pl.multiple_of((p & 3) * 1024, 1024), 1024))
        return pltpu.make_async_copy(wq_hbm.at[idx], wq_v.at[idx], sem.at[S_WQ])

    def issue_round(t, piece, nrun=16, nround=_NR, skew=None):
        skew = _SKEW if skew is None else skew
        for j in range(nrun):
            n = j - skew if j % 4 == 0 else j
            back = -(n // nrun)
            p = t if back == 0 else jnp.where(t < back, t + (nround - back), t - back)
            piece(n % nrun, p).start(priority=int(j % 4 != 0))

    def round_w(t):
        parts = (wq_piece, rows_piece(bwq_hbm, bwq_v, S_BWQ, 64),
                 rows_piece(bwuk_hbm, bwuk_v, S_BWUK, 64), rows_piece(bwuv_hbm, bwuv_v, S_BWUV, 64))
        issue_round(t, lambda r, p: parts[_WORD[r // 4]](r % 4, p))

    def round_c(t):
        issue_round(t, rows_piece(ckv_hbm, ckv_v, S_CKV, 16))

    def round_k(w, t):
        issue_round(t, rows_piece(k_hbm, k_v, S_K, 64, pl.multiple_of(w * (_HW * _SK), _HW * _SK)))

    def round_v(w, t):
        issue_round(t, rows_piece(v_hbm, v_v, S_V, 64, pl.multiple_of(w * (_HW * _SK), _HW * _SK)))

    end_lo = [0] + [48 + sum(_END[:e]) for e in range(len(_END) + 1)]

    def end_piece(e, i, u, p):
        return pltpu.make_async_copy(
            (wo_hbm, bwo_hbm)[u // 4].at[pl.ds(pl.multiple_of((u % 4) * 1024 + i * _DH + p * 16, 16), 16)],
            wob_v.at[8 * i + u, pl.ds(pl.multiple_of(p * 16, 16), 16)], sem.at[S_END + e])

    def round_end(t):
        issue_round(t, lambda u, p: end_piece(0, p >> 3, u, p & 7), nrun=8, nround=48, skew=_ESKEW)

    def wait_all(dst, s):
        pltpu.make_async_copy(dst, dst, sem.at[s]).wait()

    row8 = jax.lax.broadcasted_iota(jnp.int32, (8, _D), 0)
    row8h = jax.lax.broadcasted_iota(jnp.int32, (8, _DH), 0)
    scale = _DH ** -0.5

    def qa_step(x8, g):
        q = _dot(x8, wq_v[:, pl.ds(pl.multiple_of(g * 512, 512), 512)]) * scale
        for j in range(4):
            qa_s[4 * g + j] = q[:, j * _DH:(j + 1) * _DH]

    def words_step(w_v, blk):
        R = 512
        w32[pl.ds(pl.multiple_of(blk * R, R), R), :] = pltpu.bitcast(
            w_v[pl.ds(pl.multiple_of(2 * blk * R, 2 * R), 2 * R), :], jnp.int32)

    def head_pair(i):
        return _unpack_pair(w32[pl.ds(i, _D, stride=_H // 2), :])

    def qb_step(x8, i):
        lo, hi = head_pair(i)
        qb_s[2 * i] = _dot(x8, lo)
        qb_s[2 * i + 1] = _dot(x8, hi)

    def qlat_step(i):
        pair = head_pair(i)
        for j in range(2):
            h = 2 * i + j
            ql = _dot_t(qb_s[h].astype(_bf16), pair[j]) * scale
            qlat_s[0, pl.ds(h, 1), :] = ql[0:1, :]
            qlat_s[1, pl.ds(h, 1), :] = ql[1:2, :]

    def b_step(i):
        b = i & 1
        ck = ckv_v[pl.ds(pl.multiple_of(b * _SK + (i >> 1) * _CK, _CK), _CK), :]
        s = _dot_t(qlat_s[b].astype(_bf16), ck)
        m_old = m_s[b]
        m_new = jnp.maximum(m_old, jnp.max(s, axis=-1, keepdims=True))
        p = jnp.exp(s - m_new)
        alpha = jnp.exp(m_old - m_new)
        m_s[b] = m_new
        l_s[b] = alpha * l_s[b] + jnp.sum(p, axis=-1, keepdims=True)
        acc_s[b] = alpha * acc_s[b] + _dot(p.astype(_bf16), ck)

    def ctx_step(i):
        pair = head_pair(i)
        for j in range(2):
            h = 2 * i + j
            r0 = clat_s[0, pl.ds(h, 1), :]
            r1 = clat_s[1, pl.ds(h, 1), :]
            lhs = jnp.where(row8 == 0, r0, jnp.where(row8 == 1, r1, 0.0))
            ctx_s[h] = _dot(lhs.astype(_bf16), pair[j])

    def keys(i):
        return pl.ds(pl.multiple_of(i * _SK, _SK), _SK)

    def qk_step(w, i):
        h = (w * _HW + i) & (_H - 1)
        s = _dot_t(qa_s[h].astype(_bf16), k_v[keys(i), :])
        p = jnp.exp(s - jnp.max(s, axis=-1, keepdims=True))
        la_s[i] = jnp.broadcast_to(jnp.sum(p, axis=-1, keepdims=True), (8, _DH))
        p_s[i] = p

    def pv_step(w, i):
        bh = w * _HW + i
        b, h = bh >> 5, bh & (_H - 1)
        o = _dot(p_s[i].astype(_bf16), v_v[keys(i), :]) / la_s[i]
        o_s[h] = jnp.where(row8h == b, o, o_s[h])

    def with_rounds(issue, t0, n, per, step):
        def body(i):
            for u in range(per):
                issue(t0 + i * per + u)
            step(i)
        _loop(0, n, body)
        return t0 + n * per

    cx = pltpu.make_async_copy(x_hbm, x_ref, sem.at[S_X])
    cg = pltpu.make_async_copy(gw_hbm, gw_ref, sem.at[S_GW])
    round_w(0)
    cx.start()
    cg.start()
    _loop(1, _NR, round_w)
    o_s[...] = jnp.zeros_like(o_s)
    m_s[...] = jnp.full_like(m_s, -jnp.inf)
    l_s[...] = jnp.zeros_like(l_s)
    acc_s[...] = jnp.zeros_like(acc_s)
    cx.wait()
    cg.wait()
    xf = x_ref[...].astype(_f32)
    x8f = jnp.where(row8 == 0, xf[0:1], jnp.where(row8 == 1, xf[1:2], 0.0))
    x8 = x8f.astype(_bf16)
    gate = jax.nn.sigmoid(jnp.sum(x8f * gw_ref[...].astype(_f32).reshape(1, _D), axis=-1, keepdims=True))

    _loop(0, _LAG, round_c)
    wait_all(wq_v, S_WQ)
    wait_all(bwq_v, S_BWQ)
    wait_all(bwuk_v, S_BWUK)
    wait_all(bwuv_v, S_BWUV)
    t = with_rounds(round_c, _LAG, 8, 1, lambda g: qa_step(x8, g))
    t = with_rounds(round_c, t, 16, 1, lambda i: words_step(bwq_v, i))
    t = with_rounds(round_c, t, 16, 1, lambda i: qb_step(x8, i))
    _loop(t, _NR, round_c)

    t0 = _LAG + _RH * _HW
    nb = _SK // _CK

    def kv_windows(w):
        issue = lambda t: round_k(w, t)
        _loop(0, _LAG, issue)

        @pl.when(w == 0)
        def _():
            _loop(_LAG, t0, issue)
            t = with_rounds(issue, t0, 16, 1, lambda i: words_step(bwuk_v, i))
            with_rounds(issue, t, 16, 1, qlat_step)

        @pl.when(w > 0)
        def _():
            wait_all(v_v, S_V)
            with_rounds(issue, _LAG, _HW, _RH, lambda i: pv_step(w - 1, i))

        @pl.when(w == 1)
        def _():
            with_rounds(issue, t0, nb, 32 // nb, lambda i: b_step(nb + i))

        _loop(jnp.where(w <= 1, t0 + 32, t0), _NR, issue)

        issue = lambda t: round_v(w, t)
        _loop(0, _LAG, issue)
        wait_all(k_v, S_K)
        with_rounds(issue, _LAG, _HW, _RH, lambda i: qk_step(w, i))

        @pl.when(w == 0)
        def _():
            wait_all(ckv_v, S_CKV)
            with_rounds(issue, t0, nb, 32 // nb, b_step)

        @pl.when(w == 1)
        def _():
            clat_s[...] = acc_s[...] / l_s[...]
            t = with_rounds(issue, t0, 16, 1, lambda i: words_step(bwuv_v, i))
            with_rounds(issue, t, 16, 1, ctx_step)

        _loop(jnp.where(w <= 1, t0 + 32, t0), _NR, issue)

    NW = _B * _H // _HW
    _loop(0, NW, kv_windows)

    _loop(0, 2 * _LAG, round_end)
    wait_all(v_v, S_V)
    with_rounds(round_end, 2 * _LAG, _HW, (48 - 2 * _LAG) // _HW, lambda i: pv_step(NW - 1, i))
    for e in range(1, len(_END) + 1):
        n = 0
        for p in range(8):
            for q in range(end_lo[e], end_lo[e + 1]):
                end_piece(e, q // 8, q % 8, p).start(priority=int(_EPRIO[e][n % len(_EPRIO[e])]))
                n += 1

    acc = [None, None]
    for e in range(len(_END) + 1):
        wait_all(wob_v.at[pl.ds(end_lo[e], end_lo[e + 1] - end_lo[e])], S_END + e)
        for q in range(end_lo[e], end_lo[e + 1]):
            i, j, r = q // 8, (q % 8) // 4, q % 4
            t = _dot((o_s, ctx_s)[j][8 * r + i].astype(_bf16), wob_v[q])
            acc[j] = t if acc[j] is None else acc[j] + t
    res = gate * acc[0] + (1.0 - gate) * acc[1]
    out_ref[...] = res[0:2, :].astype(_bf16)


@jax.jit
def pallas_gated_mix__mha_block_cached__compressed_kv_cla__decode_kernel(
    A_x: jax.Array,
    A_k_cache: jax.Array,
    A_v_cache: jax.Array,
    A_wq: jax.Array,
    A_wo: jax.Array,
    B_x: jax.Array,
    B_c_kv: jax.Array,
    B_w_q: jax.Array,
    B_w_uk: jax.Array,
    B_w_uv: jax.Array,
    B_w_o: jax.Array,
    gate_w: jax.Array,
):
    del B_x
    k2 = A_k_cache.reshape(_B * _H * _SK, _DH)
    v2 = A_v_cache.reshape(_B * _H * _SK, _DH)
    ckv = B_c_kv.reshape(_B * _SK, _DC)
    bwq = B_w_q.reshape(_D * _H, _DH)
    bwuk = B_w_uk.reshape(_DC * _H, _DH)
    bwuv = B_w_uv.reshape(_DC * _H, _DH)
    bwo = B_w_o.reshape(_H * _DH, _D)
    x2 = A_x.reshape(_B, _D)

    hbm = pl.BlockSpec(memory_space=pl.ANY)
    vmem = pl.BlockSpec(memory_space=pltpu.VMEM)
    V = pltpu.VMEM
    scratch = [
        V((_HW * _SK, _DH), _bf16),
        V((_HW * _SK, _DH), _bf16),
        V((_D, _H * _DH), _bf16),
        V((2 * _H, _DH, _D), _bf16),
        V((_B * _SK, _DC), _bf16),
        V((_D * _H, _DH), _bf16),
        V((_DC * _H, _DH), _bf16),
        V((_DC * _H, _DH), _bf16),
        V((_H, 8, _DH), _f32),
        V((_HW, 8, _SK), _f32),
        V((_HW, 8, _DH), _f32),
        V((_H, 8, _DH), _f32),
        V((_B, _H, _DC), _f32),
        V((_B, _H, _DC), _f32),
        V((_H, 8, _DH), _f32),
        V((_H, 8, _DH), _f32),
        V((_B, _H, 1), _f32),
        V((_B, _H, 1), _f32),
        V((_B, _H, _DC), _f32),
        V((_B, _D), _bf16),
        V((_D,), _bf16),
        V((_D * _H // 2, _DH), jnp.int32),
        pltpu.SemaphoreType.DMA((10 + len(_END),)),
    ]
    out = pl.pallas_call(
        _kernel,
        out_shape=jax.ShapeDtypeStruct((_B, _D), _bf16),
        in_specs=[hbm] * 11,
        out_specs=vmem,
        scratch_shapes=scratch,
        compiler_params=pltpu.CompilerParams(vmem_limit_bytes=100 * 1024 * 1024,
                                             disable_semaphore_checks=True),
    )(x2, gate_w, k2, v2, A_wq, A_wo, ckv, bwq, bwuk, bwuv, bwo)
    return out.reshape(_B, 1, _D)
```

```python
import jax
import jax.numpy as jnp
import jax.experimental.pallas as pl
import jax.experimental.pallas.tpu as pltpu

_B, _H, _SK, _DH, _D, _DC = 2, 32, 8192, 128, 512, 512

_NR = 64
_HW = 8
_SKEW = 32
_LAG = 16
_CK = 1024
_END = (48, 8, 4, 2, 2)

_f32 = jnp.float32
_bf16 = jnp.bfloat16


def _dot(a, b):
    return jnp.dot(a, b, preferred_element_type=_f32)


def _dot_t(a, b):
    return jax.lax.dot_general(a, b, (((1,), (1,)), ((), ())), preferred_element_type=_f32)


def _unpack_pair(blk):
    lo = pltpu.bitcast(blk << 16, _f32).astype(_bf16)
    hi = pltpu.bitcast(blk & jnp.int32(-65536), _f32).astype(_bf16)
    return lo, hi


def _loop(lo, hi, body):
    def step(i, carry):
        body(i)
        return carry
    jax.lax.fori_loop(lo, hi, step, 0)


def _kernel(x_hbm, gw_hbm,
            k_hbm, v_hbm, wq_hbm, wo_hbm, ckv_hbm, bwq_hbm, bwuk_hbm, bwuv_hbm, bwo_hbm,
            out_ref,
            k_v, v_v, wq_v, wob_v, ckv_v, bwq_v, bwuk_v, bwuv_v,
            qa_s, p_s, la_s, qb_s, qlat_s, clat_s, o_s, ctx_s, m_s, l_s, acc_s,
            x_ref, gw_ref, w32, sem):

    S_X, S_GW, S_K, S_V, S_WQ, S_BWQ, S_BWUK, S_BWUV, S_CKV, S_END = range(10)

    def rows_piece(src, dst, s, nrow, src0=0):
        def piece(r, p):
            row = pl.multiple_of((r * _NR + p) * nrow, nrow)
            return pltpu.make_async_copy(src.at[pl.ds(src0 + row, nrow)], dst.at[pl.ds(row, nrow)], sem.at[s])
        return piece

    def wq_piece(r, p):
        idx = (r * 16 + (p >> 2), slice(None), pl.ds(pl.multiple_of((p & 3) * 1024, 1024), 1024))
        return pltpu.make_async_copy(wq_hbm.at[idx], wq_v.at[idx], sem.at[S_WQ])

    w_parts = (wq_piece, rows_piece(bwq_hbm, bwq_v, S_BWQ, 64),
               rows_piece(bwuk_hbm, bwuk_v, S_BWUK, 64), rows_piece(bwuv_hbm, bwuv_v, S_BWUV, 64))

    def w_piece(r, p):
        return w_parts[r // 4](r % 4, p)

    c_piece = rows_piece(ckv_hbm, ckv_v, S_CKV, 16)

    def k_piece(w):
        return rows_piece(k_hbm, k_v, S_K, 64, pl.multiple_of(w * (_HW * _SK), _HW * _SK))

    def v_piece(w):
        return rows_piece(v_hbm, v_v, S_V, 64, pl.multiple_of(w * (_HW * _SK), _HW * _SK))

    def end_piece(e, i, u, p):
        return pltpu.make_async_copy(
            (wo_hbm, bwo_hbm)[u // 4].at[pl.ds(pl.multiple_of((u % 4) * 1024 + i * _DH + p * 16, 16), 16)],
            wob_v.at[8 * i + u, pl.ds(pl.multiple_of(p * 16, 16), 16)], sem.at[S_END + e])

    def e_piece(u, p):
        return end_piece(0, p >> 3, u, p & 7)

    def issue_round(piece, t, nrun=16, prev=None):
        back = _SKEW // nrun
        for j in range(nrun):
            if j % 4:
                piece(j, t).start(priority=1)
            elif not isinstance(t, int) or t >= back:
                piece(j, t - back).start(priority=0)
            elif prev is not None:
                n = t * nrun + j
                prev(n % 16, _NR - _SKEW // 16 + n // 16).start(priority=0)

    def start_window(piece, prev, end, nrun=16):
        for t in range(_SKEW // nrun):
            issue_round(piece, t, nrun, prev)
        _loop(_SKEW // nrun, end, lambda t: issue_round(piece, t, nrun))

    def wait_all(dst, s):
        pltpu.make_async_copy(dst, dst, sem.at[s]).wait()

    def with_rounds(issue, t0, n, per, step):
        def body(i):
            for u in range(per):
                issue(t0 + i * per + u)
            step(i)
        _loop(0, n, body)
        return t0 + n * per

    row8 = jax.lax.broadcasted_iota(jnp.int32, (8, _D), 0)
    row8h = jax.lax.broadcasted_iota(jnp.int32, (8, _DH), 0)
    scale = _DH ** -0.5

    def qa_step(x8, g):
        w = wq_v[:, :, pl.ds(pl.multiple_of(g * 512, 512), 512)]
        q = _dot(x8, w.astype(_f32).reshape(_D, 512).astype(_bf16)) * scale
        for j in range(4):
            qa_s[4 * g + j] = q[:, j * _DH:(j + 1) * _DH]

    def words_step(w_v, blk):
        R = 1024
        w32[pl.ds(pl.multiple_of(blk * R, R), R), :] = pltpu.bitcast(
            w_v[pl.ds(pl.multiple_of(2 * blk * R, 2 * R), 2 * R), :], jnp.int32)

    def head_pair(i):
        return _unpack_pair(w32[pl.ds(i, _D, stride=_H // 2), :])

    def qb_step(x8, i):
        lo, hi = head_pair(i)
        qb_s[2 * i] = _dot(x8, lo)
        qb_s[2 * i + 1] = _dot(x8, hi)

    def qlat_step(i):
        pair = head_pair(i)
        for j in range(2):
            h = 2 * i + j
            ql = _dot_t(qb_s[h].astype(_bf16), pair[j]) * scale
            qlat_s[0, pl.ds(h, 1), :] = ql[0:1, :]
            qlat_s[1, pl.ds(h, 1), :] = ql[1:2, :]

    def b_step(i, between):
        b = i & 1
        rows = pl.ds(pl.multiple_of(b * _SK + (i >> 1) * _CK, _CK), _CK)
        between(0)
        s = _dot_t(qlat_s[b].astype(_bf16), ckv_v[rows, :])
        between(1)
        m_old = m_s[b]
        m_new = jnp.maximum(m_old, jnp.max(s, axis=-1, keepdims=True))
        p = jnp.exp(s - m_new)
        alpha = jnp.exp(m_old - m_new)
        m_s[b] = m_new
        l_s[b] = alpha * l_s[b] + jnp.sum(p, axis=-1, keepdims=True)
        acc_s[b] = alpha * acc_s[b] + _dot(p.astype(_bf16), ckv_v[rows, :])

    def ctx_step(i):
        pair = head_pair(i)
        for j in range(2):
            h = 2 * i + j
            r0 = clat_s[0, pl.ds(h, 1), :]
            r1 = clat_s[1, pl.ds(h, 1), :]
            lhs = jnp.where(row8 == 0, r0, jnp.where(row8 == 1, r1, 0.0))
            ctx_s[h] = _dot(lhs.astype(_bf16), pair[j])

    def qk_step(w, i, between):
        h = (w * _HW + i) & (_H - 1)
        q = qa_s[h].astype(_bf16)
        n = _SK // 2
        s = []
        for u in range(2):
            between(u)
            s.append(_dot_t(q, k_v[pl.ds(pl.multiple_of(i * _SK + u * n, n), n), :]))
        s = jnp.concatenate(s, axis=-1)
        p = jnp.exp(s - jnp.max(s, axis=-1, keepdims=True))
        la_s[i] = jnp.broadcast_to(jnp.sum(p, axis=-1, keepdims=True), (8, _DH))
        p_s[i] = p

    def pv_step(w, i):
        bh = w * _HW + i
        b, h = bh >> 5, bh & (_H - 1)
        v = v_v[pl.ds(pl.multiple_of(i * _SK, _SK), _SK), :]
        o = _dot(p_s[i].astype(_bf16), v) / la_s[i]
        o_s[h] = jnp.where(row8h == b, o, o_s[h])

    def per_head_pair(issue, t, w_v, step):
        t = with_rounds(issue, t, 8, 1, lambda i: words_step(w_v, i))
        return with_rounds(issue, t, 16, 1, step)

    cx = pltpu.make_async_copy(x_hbm, x_ref, sem.at[S_X])
    cg = pltpu.make_async_copy(gw_hbm, gw_ref, sem.at[S_GW])
    start_window(w_piece, None, _LAG)
    cx.start()
    cg.start()
    _loop(_LAG, _NR, lambda t: issue_round(w_piece, t))
    o_s[...] = jnp.zeros_like(o_s)
    m_s[...] = jnp.full_like(m_s, -jnp.inf)
    l_s[...] = jnp.zeros_like(l_s)
    acc_s[...] = jnp.zeros_like(acc_s)
    cx.wait()
    cg.wait()
    xf = x_ref[...].astype(_f32)
    x8f = jnp.where(row8 == 0, xf[0:1], jnp.where(row8 == 1, xf[1:2], 0.0))
    x8 = x8f.astype(_bf16)
    gate = jax.nn.sigmoid(jnp.sum(x8f * gw_ref[...].astype(_f32).reshape(1, _D), axis=-1, keepdims=True))

    issue = lambda t: issue_round(c_piece, t)
    start_window(c_piece, w_piece, _LAG)
    wait_all(wq_v, S_WQ)
    wait_all(bwq_v, S_BWQ)
    wait_all(bwuk_v, S_BWUK)
    wait_all(bwuv_v, S_BWUV)
    t = with_rounds(issue, _LAG, 8, 1, lambda g: qa_step(x8, g))
    t = per_head_pair(issue, t, bwq_v, lambda i: qb_step(x8, i))
    _loop(t, _NR, issue)

    t0 = _LAG + 3 * _HW
    assert t0 + 24 == _NR

    def kv_windows(w):
        issue = lambda t: issue_round(k_piece(w), t)

        @pl.when(w == 0)
        def _():
            start_window(k_piece(w), c_piece, t0)
            per_head_pair(issue, t0, bwuk_v, qlat_step)
            wait_all(ckv_v, S_CKV)

        @pl.when(w > 0)
        def _():
            start_window(k_piece(w), v_piece(w - 1), _LAG)
            wait_all(v_v, S_V)
            with_rounds(issue, _LAG, _HW, 3, lambda i: pv_step(w - 1, i))
            _loop(t0, _NR, issue)

        issue = lambda t: issue_round(v_piece(w), t)
        start_window(v_piece(w), k_piece(w), _LAG)
        wait_all(k_v, S_K)

        def head(i):
            def between(u):
                for r in ((0, 1), (2,))[u]:
                    issue(_LAG + 3 * i + r)
            qk_step(w, i, between)
        _loop(0, _HW, head)

        @pl.when(w < 4)
        def _():
            def chunk(i):
                def between(u):
                    for r in range(3):
                        issue(t0 + 6 * i + 3 * u + r)
                b_step(4 * w + i, between)
            _loop(0, 4, chunk)

        @pl.when(w == 4)
        def _():
            clat_s[...] = acc_s[...] / l_s[...]
            per_head_pair(issue, t0, bwuv_v, ctx_step)

        @pl.when(w > 4)
        def _():
            _loop(t0, _NR, issue)

    NW = _B * _H // _HW
    assert 4 * 4 * _CK == _B * _SK
    _loop(0, NW, kv_windows)

    issue = lambda t: issue_round(e_piece, t, nrun=8)
    start_window(e_piece, v_piece(NW - 1), 24, nrun=8)
    wait_all(v_v, S_V)
    t = with_rounds(issue, 24, _HW, 3, lambda i: pv_step(NW - 1, i))
    assert t == _END[0]
    lo = [sum(_END[:e]) for e in range(len(_END) + 1)]
    last = [(0, p >> 3, u, p & 7) for p in range(t - _SKEW // 8, t) for u in range(8)]
    last += [(e, q // 8, q % 8, p) for e in range(1, len(_END)) for p in range(8) for q in range(lo[e], lo[e + 1])]
    for n in range(_SKEW, len(last) + _SKEW):
        if n % 4 == 0:
            end_piece(*last[n - _SKEW]).start(priority=0)
        elif n < len(last):
            end_piece(*last[n]).start(priority=1)

    acc = [None, None]
    for e in range(len(_END)):
        wait_all(wob_v.at[pl.ds(lo[e], _END[e])], S_END + e)
        for q in range(lo[e], lo[e + 1]):
            i, j, r = q // 8, (q % 8) // 4, q % 4
            part = _dot((o_s, ctx_s)[j][8 * r + i].astype(_bf16), wob_v[q])
            acc[j] = part if acc[j] is None else acc[j] + part
    res = gate * acc[0] + (1.0 - gate) * acc[1]
    out_ref[...] = res[0:2, :].astype(_bf16)


@jax.jit
def pallas_gated_mix__mha_block_cached__compressed_kv_cla__decode_kernel(
    A_x: jax.Array,
    A_k_cache: jax.Array,
    A_v_cache: jax.Array,
    A_wq: jax.Array,
    A_wo: jax.Array,
    B_x: jax.Array,
    B_c_kv: jax.Array,
    B_w_q: jax.Array,
    B_w_uk: jax.Array,
    B_w_uv: jax.Array,
    B_w_o: jax.Array,
    gate_w: jax.Array,
):
    del B_x
    k2 = A_k_cache.reshape(_B * _H * _SK, _DH)
    v2 = A_v_cache.reshape(_B * _H * _SK, _DH)
    wq3 = A_wq.reshape(_D // 8, 8, _H * _DH)
    ckv = B_c_kv.reshape(_B * _SK, _DC)
    bwq = B_w_q.reshape(_D * _H, _DH)
    bwuk = B_w_uk.reshape(_DC * _H, _DH)
    bwuv = B_w_uv.reshape(_DC * _H, _DH)
    bwo = B_w_o.reshape(_H * _DH, _D)
    x2 = A_x.reshape(_B, _D)

    hbm = pl.BlockSpec(memory_space=pl.ANY)
    vmem = pl.BlockSpec(memory_space=pltpu.VMEM)
    V = pltpu.VMEM
    scratch = [
        V((_HW * _SK, _DH), _bf16),
        V((_HW * _SK, _DH), _bf16),
        V((_D // 8, 8, _H * _DH), _bf16),
        V((2 * _H, _DH, _D), _bf16),
        V((_B * _SK, _DC), _bf16),
        V((_D * _H, _DH), _bf16),
        V((_DC * _H, _DH), _bf16),
        V((_DC * _H, _DH), _bf16),
        V((_H, 8, _DH), _f32),
        V((_HW, 8, _SK), _f32),
        V((_HW, 8, _DH), _f32),
        V((_H, 8, _DH), _f32),
        V((_B, _H, _DC), _f32),
        V((_B, _H, _DC), _f32),
        V((_H, 8, _DH), _f32),
        V((_H, 8, _DH), _f32),
        V((_B, _H, 1), _f32),
        V((_B, _H, 1), _f32),
        V((_B, _H, _DC), _f32),
        V((_B, _D), _bf16),
        V((_D,), _bf16),
        V((_D * _H // 2, _DH), jnp.int32),
        pltpu.SemaphoreType.DMA((9 + len(_END),)),
    ]
    out = pl.pallas_call(
        _kernel,
        out_shape=jax.ShapeDtypeStruct((_B, _D), _bf16),
        in_specs=[hbm] * 11,
        out_specs=vmem,
        scratch_shapes=scratch,
        compiler_params=pltpu.CompilerParams(vmem_limit_bytes=100 * 1024 * 1024,
                                             disable_semaphore_checks=True),
    )(x2, gate_w, k2, v2, wq3, A_wo, ckv, bwq, bwuk, bwuv, bwo)
    return out.reshape(_B, 1, _D)
```
